```python
import os as _os
_os.environ.setdefault("JAX_PLATFORMS", "cpu")
import jax
import jax.numpy as jnp

def _softmax(x, axis=-1):
    return jax.nn.softmax(x, axis=axis)
def _gelu(x):
    return jax.nn.gelu(x, approximate=True)
def _silu(x):
    return jax.nn.silu(x)
def _sigmoid(x):
    return jax.nn.sigmoid(x)
def _layernorm(x, axis=-1, eps=1e-5):
    m = jnp.mean(x, axis=axis, keepdims=True)
    v = jnp.var(x, axis=axis, keepdims=True)
    return (x - m) / jnp.sqrt(v + eps)
def _scatter_add(tgt, idx, src, axis=0):
    return tgt.at[idx].add(src)
def _segment_sum(src, seg, n):
    return jax.ops.segment_sum(src, seg, n)
class _Rng:
    def __init__(self, key):
        self._k = key
    def _next(self):
        self._k, sub = jax.random.split(self._k)
        return sub
    def normal(self, shape):
        return jax.random.normal(self._next(), shape, dtype=jnp.bfloat16)
    def randint(self, lo, hi, shape):
        return jax.random.randint(self._next(), shape, lo, hi, dtype=jnp.int32)
    def uniform(self, shape, lo=0.0, hi=1.0):
        return jax.random.uniform(self._next(), shape, jnp.bfloat16, lo, hi)
    def permutation(self, n):
        return jax.random.permutation(self._next(), n)


kernel_name = 'standalone__gqa_block_cached__near_ridge'

def setup_inputs():
    _rng = _Rng(jax.random.key(int.from_bytes(__import__("os").urandom(4), "little")))
    _w = (lambda a: (lambda t: t.astype(jnp.bfloat16) if jnp.issubdtype(t.dtype, jnp.floating) else t)(jnp.asarray(a)))
    B, Sq, D = 8, 96, 448
    Hq, Hkv, Sk, Dh = 16, 8, 2048, 256
    assert Hq % Hkv == 0, (Hq, Hkv)
    return {
        "x": _w((lambda *s: _rng.normal(s) * 0.8)(B, Sq, D)),
        "k_cache": _w((lambda *s: _rng.normal(s) * 0.8)(B, Hkv, Sk, Dh)),
        "v_cache": _w((lambda *s: _rng.normal(s) * 0.05)(B, Hkv, Sk, Dh)),
        "wq": _w((lambda *s: _rng.normal(s) * 0.8)(D, Hq * Dh) * (D ** -0.5)),
        "wo": _w((lambda *s: _rng.normal(s) * 0.05)(Hq * Dh, D) * ((Hq * Dh) ** -0.5)),
    }

def reference(x, k_cache, v_cache, wq, wo):
    B, Sq, D = x.shape
    Hq, Dh = 16, 256
    Hkv = k_cache.shape[1]
    rep = Hq // Hkv
    q = (lambda x, *d: x.transpose(*d))((x @ wq).reshape(B, Sq, Hq, Dh), 0, 2, 1, 3)
    k = jnp.repeat(k_cache, rep, axis=1)
    v = jnp.repeat(v_cache, rep, axis=1)
    scores = jnp.einsum("bhqd,bhkd->bhqk", q, k) * (Dh ** -0.5)
    p = _softmax(scores, axis=-1)
    o = jnp.einsum("bhqk,bhkd->bhqd", p, v)
    return (lambda x, *d: x.transpose(*d))(o, 0, 2, 1, 3).reshape(B, Sq, Hq * Dh) @ wo
```

```python
import functools
import math

import jax
import jax.numpy as jnp
import jax.experimental.pallas as pl
import jax.experimental.pallas.tpu as pltpu

HQ = 16
DH = 256


def _kernel(x_ref, k_ref, v_ref, wq_ref, wo_ref, o_ref, q_scr, oall_scr, acc_scr,
            *, B, Sq, rep, scale):
    h = pl.program_id(0)
    b = pl.program_id(1)
    nh = pl.num_programs(0)

    @pl.when(b == 0)
    def _():
        q = jnp.dot(x_ref[...], wq_ref[...], preferred_element_type=jnp.float32)
        qb = q.astype(jnp.bfloat16)
        for bb in range(B):
            for r in range(rep):
                q_scr[bb, r * Sq:(r + 1) * Sq, :] = qb[bb * Sq:(bb + 1) * Sq, r * DH:(r + 1) * DH]

    q = q_scr[b]
    k = k_ref[0, 0]
    v = v_ref[0, 0]
    s = jax.lax.dot_general(q, k, (((1,), (1,)), ((), ())),
                            preferred_element_type=jnp.float32)
    s = s * scale
    m = jnp.max(s, axis=-1, keepdims=True)
    p = jnp.exp(s - m)
    l = jnp.sum(p, axis=-1, keepdims=True)
    o = jnp.dot(p.astype(jnp.bfloat16), v, preferred_element_type=jnp.float32)
    o = (o / l).astype(jnp.bfloat16)
    for r in range(rep):
        oall_scr[b, :, r * DH:(r + 1) * DH] = o[r * Sq:(r + 1) * Sq, :]

    @pl.when(b == B - 1)
    def _():
        oa = oall_scr[...].reshape(B * Sq, rep * DH)
        contrib = jnp.dot(oa, wo_ref[...], preferred_element_type=jnp.float32)

        @pl.when(h == 0)
        def _():
            acc_scr[...] = contrib

        @pl.when(h > 0)
        def _():
            acc_scr[...] += contrib

        @pl.when(h == nh - 1)
        def _():
            o_ref[...] = acc_scr[...].astype(o_ref.dtype)


@jax.jit
def pallas_standalone__gqa_block_cached__near_ridge_kernel(
    x: jax.Array,
    k_cache: jax.Array,
    v_cache: jax.Array,
    wq: jax.Array,
    wo: jax.Array,
):
    B, Sq, D = x.shape
    _, Hkv, Sk, Dh = k_cache.shape
    assert Dh == DH
    rep = HQ // Hkv
    scale = float(Dh) ** -0.5
    x2 = x.reshape(B * Sq, D)

    kern = functools.partial(_kernel, B=B, Sq=Sq, rep=rep, scale=scale)
    out = pl.pallas_call(
        kern,
        grid=(Hkv, B),
        in_specs=[
            pl.BlockSpec((B * Sq, D), lambda h, b: (0, 0)),
            pl.BlockSpec((1, 1, Sk, Dh), lambda h, b: (b, h, 0, 0)),
            pl.BlockSpec((1, 1, Sk, Dh), lambda h, b: (b, h, 0, 0)),
            pl.BlockSpec((D, rep * Dh), lambda h, b: (0, h)),
            pl.BlockSpec((rep * Dh, D), lambda h, b: (h, 0)),
        ],
        out_specs=pl.BlockSpec((B * Sq, D), lambda h, b: (0, 0)),
        out_shape=jax.ShapeDtypeStruct((B * Sq, D), x.dtype),
        scratch_shapes=[
            pltpu.VMEM((B, rep * Sq, Dh), jnp.bfloat16),
            pltpu.VMEM((B, Sq, rep * Dh), jnp.bfloat16),
            pltpu.VMEM((B * Sq, D), jnp.float32),
        ],
        compiler_params=pltpu.CompilerParams(
            dimension_semantics=("arbitrary", "arbitrary"),
            vmem_limit_bytes=96 * 1024 * 1024,
        ),
    )(x2, k_cache, v_cache, wq, wo)
    return out.reshape(B, Sq, D)
```

```python
import functools

import jax
import jax.numpy as jnp
import jax.experimental.pallas as pl
import jax.experimental.pallas.tpu as pltpu

HQ = 16
DH = 256
NB = 8
LEAD = 1
NSB = LEAD + 1
U = 2
CK = 512
SUB = 64
WSUB = 32
LA = 4
NODMA = 0
BLK = 0
GW = 1
assert U % GW == 0
assert U % NSB == 0


def _divmod_pow2(t, n):
    assert n & (n - 1) == 0
    if isinstance(t, int):
        return t // n, t % n
    sh = n.bit_length() - 1
    return jax.lax.shift_right_logical(t, sh), jax.lax.bitwise_and(t, n - 1)


def _kernel(x_hbm, k_hbm, v_hbm, wq_hbm, wo_hbm, out_hbm,
            xbuf, wqbuf, wobuf, kbuf, vbuf, acc, obuf, *rest,
            B, Sq, Hkv, Sk, D, rep, scale):
    sbufs = rest[:NSB]
    mbufs = rest[NSB:2 * NSB]
    xsem, wqsem, wosem, ksem, vsem, osem = rest[2 * NSB:]
    T = B * Hkv
    W = rep * DH
    M = rep * Sq
    NC = Sk // CK
    NS = CK // SUB
    f32 = jnp.float32
    bf16 = jnp.bfloat16

    def hb(t):
        return _divmod_pow2(t, B)

    def slot_of(t):
        return _divmod_pow2(t, NB)[1]

    def when(cond, fn):
        if isinstance(cond, bool):
            if cond:
                fn()
        else:
            pl.when(cond)(fn)

    def land(a, b):
        if isinstance(a, bool) and isinstance(b, bool):
            return a and b
        return jnp.logical_and(a, b)

    def blk_copy(hbm, buf, sem, t, r0, nrows):
        h, b = hb(t)
        slot = slot_of(t)
        return pltpu.make_async_copy(hbm.at[b, h, pl.ds(r0, nrows)], buf.at[slot, pl.ds(r0, nrows)],
                                     sem.at[slot])

    def w_copy(hbm, buf, sem, h, r0, nrows):
        return pltpu.make_async_copy(hbm.at[pl.ds(r0, nrows), pl.ds(h * W, W)], buf.at[h, pl.ds(r0, nrows)],
                                     sem.at[h])

    def issue_d(p, c):
        tk = p + LEAD
        tv = p
        static = isinstance(p, int)
        k_ok = tk < T
        v_ok = (0 <= tv < T) if static else tv < T
        if static and not k_ok and not v_ok:
            return
        hk, bk = hb(tk)
        hv, bv = hb(max(tv, 0) if static else tv)
        if c == 0:
            for i, r0 in enumerate(range(0, D, WSUB)):
                when(land(k_ok, bk == 0), lambda: w_copy(wq_hbm, wqbuf, wqsem, hk, r0, WSUB).start(priority=i % 2))
        if c == NC - 1:
            for i, r0 in enumerate(range(0, D, WSUB)):
                when(land(v_ok, bv == 0), lambda: w_copy(wo_hbm, wobuf, wosem, hv, r0, WSUB).start(priority=i % 2))
        single = static and not (k_ok and v_ok)
        if NODMA:
            return
        for j in range(NS):
            r0 = c * CK + j * SUB
            when(k_ok, lambda: blk_copy(k_hbm, kbuf, ksem, tk, r0, SUB).start(
                priority=(j % 2) if (single or BLK) else 0))
            when(v_ok, lambda: blk_copy(v_hbm, vbuf, vsem, tv, r0, SUB).start(
                priority=((j + 1) % 2) if (single or BLK) else 1))

    def wait_wq(t):
        h, b = hb(t)
        when(b == 0, lambda: w_copy(wq_hbm, wqbuf, wqsem, h, 0, D).wait())

    def wait_wo(t):
        h, b = hb(t)
        when(b == 0, lambda: w_copy(wo_hbm, wobuf, wosem, h, 0, D).wait())

    def wait_k(t):
        if not NODMA:
            blk_copy(k_hbm, kbuf, ksem, t, 0, Sk).wait()

    def wait_v(t):
        if not NODMA:
            blk_copy(v_hbm, vbuf, vsem, t, 0, Sk).wait()

    def x_copy(b):
        return pltpu.make_async_copy(x_hbm.at[b], xbuf.at[b], xsem.at[b])

    def o_copy(b):
        return pltpu.make_async_copy(obuf.at[b], out_hbm.at[b], osem.at[b])

    def q_proj(t):
        h, b = hb(t)
        q = jnp.dot(xbuf[b], wqbuf[h], preferred_element_type=f32)
        qb = (q.astype(bf16) * scale).astype(bf16)
        return jnp.concatenate([qb[:, r * DH:(r + 1) * DH] for r in range(rep)], axis=0)

    def a_chunk(t, sb, q2, c, mrun):
        slot = slot_of(t)
        kc = kbuf[slot, c * CK:(c + 1) * CK, :]
        s = jax.lax.dot_general(q2, kc, (((1,), (1,)), ((), ())), preferred_element_type=f32)
        sbufs[sb][:, c * CK:(c + 1) * CK] = s
        for j in range(CK // 128):
            sj = s[:, j * 128:(j + 1) * 128]
            mrun = sj if mrun is None else jnp.maximum(mrun, sj)
        return mrun

    def a_fin(sb, mrun):
        m = jnp.max(mrun, axis=-1, keepdims=True)
        mbufs[sb][...] = jnp.broadcast_to(m, (M, 128))

    def b_chunk(t, sb, m128, c, lrun, o):
        slot = slot_of(t)
        ps = []
        for j in range(CK // 128):
            sj = sbufs[sb][:, c * CK + j * 128:c * CK + (j + 1) * 128]
            pj = jnp.exp(sj - m128)
            lrun = pj if lrun is None else lrun + pj
            ps.append(pj.astype(bf16))
        p = jnp.concatenate(ps, axis=1)
        vc = vbuf[slot, c * CK:(c + 1) * CK, :]
        oc = jnp.dot(p, vc, preferred_element_type=f32)
        o = oc if o is None else o + oc
        return lrun, o

    def b_fin(t, lrun, o):
        h, b = hb(t)
        l = jnp.sum(lrun, axis=-1, keepdims=True)
        o = (o / l).astype(bf16)
        o2 = jnp.concatenate([o[r * Sq:(r + 1) * Sq, :] for r in range(rep)], axis=1)
        contrib = jax.lax.dot_general(o2, wobuf[h], (((1,), (1,)), ((), ())),
                                      preferred_element_type=f32)
        new = acc[b] + contrib
        acc[b] = new
        obuf[b] = new.astype(obuf.dtype)

    def issue_for(t, c):
        q = c + LA
        issue_d(t + GW + q // NC, q % NC)

    def stage(t, tmod, do_a, do_b):
        sa = (tmod + LEAD) % NSB
        sb = tmod % NSB
        if do_a:
            q2 = q_proj(t + LEAD)
        if do_b:
            m128 = mbufs[sb][...]
        mrun = None
        lrun = None
        o = None
        for c in range(NC):
            issue_for(t, c)
            if do_b:
                lrun, o = b_chunk(t, sb, m128, c, lrun, o)
            if do_a:
                mrun = a_chunk(t + LEAD, sa, q2, c, mrun)
        if do_a:
            a_fin(sa, mrun)
        if do_b:
            b_fin(t, lrun, o)

    def group(t0, n, tmod0):
        flags = []
        for j in range(n):
            t = t0 + j
            do_a = (t + LEAD < T) if isinstance(t, int) else True
            do_b = (t >= 0) if isinstance(t, int) else True
            flags.append((do_a, do_b))
            if do_a:
                wait_wq(t + LEAD)
                wait_k(t + LEAD)
            if do_b:
                wait_v(t)
                wait_wo(t)
        for j in range(n):
            stage(t0 + j, (tmod0 + j) % NSB, *flags[j])
        for j in range(n):
            if flags[j][1]:
                h, b = hb(t0 + j)
                when(h == Hkv - 1, lambda: o_copy(b).start())

    x_copy(0).start(priority=1)
    for c in range(NC):
        issue_d(-LEAD, c)
    for b in range(1, B):
        x_copy(b).start(priority=b % 2)
    acc[...] = jnp.zeros(acc.shape, acc.dtype)
    for g in range(NC, NC * GW + LA):
        issue_d(-LEAD + g // NC, g % NC)
    for b in range(B):
        x_copy(b).wait()
    for t in range(-LEAD, 0):
        group(t, 1, t % NSB)

    n_full = T - LEAD
    n_loop = n_full // U

    def body(u, carry):
        for g in range(U // GW):
            group(u * U + g * GW, GW, (g * GW) % NSB)
        return carry

    jax.lax.fori_loop(0, n_loop, body, 0)

    for t in range(n_loop * U, T):
        group(t, 1, t % NSB)
    for b in range(B):
        o_copy(b).wait()


@jax.jit
def pallas_standalone__gqa_block_cached__near_ridge_kernel(
    x: jax.Array,
    k_cache: jax.Array,
    v_cache: jax.Array,
    wq: jax.Array,
    wo: jax.Array,
):
    B, Sq, D = x.shape
    _, Hkv, Sk, Dh = k_cache.shape
    assert Dh == DH
    rep = HQ // Hkv
    W = rep * Dh
    M = rep * Sq
    scale = float(Dh) ** -0.5

    kern = functools.partial(_kernel, B=B, Sq=Sq, Hkv=Hkv, Sk=Sk, D=D, rep=rep, scale=scale)
    any_spec = pl.BlockSpec(memory_space=pl.ANY)
    out = pl.pallas_call(
        kern,
        in_specs=[any_spec] * 5,
        out_specs=any_spec,
        out_shape=jax.ShapeDtypeStruct((B, Sq, D), x.dtype),
        scratch_shapes=[
            pltpu.VMEM((B, Sq, D), jnp.bfloat16),
            pltpu.VMEM((Hkv, D, W), jnp.bfloat16),
            pltpu.VMEM((Hkv, D, W), jnp.bfloat16),
            pltpu.VMEM((NB, Sk, Dh), jnp.bfloat16),
            pltpu.VMEM((NB, Sk, Dh), jnp.bfloat16),
            pltpu.VMEM((B, Sq, D), jnp.float32),
            pltpu.VMEM((B, Sq, D), jnp.bfloat16),
        ] + [pltpu.VMEM((M, Sk), jnp.float32)] * NSB + [pltpu.VMEM((M, 128), jnp.float32)] * NSB + [
            pltpu.SemaphoreType.DMA((B,)),
            pltpu.SemaphoreType.DMA((Hkv,)),
            pltpu.SemaphoreType.DMA((Hkv,)),
            pltpu.SemaphoreType.DMA((NB,)),
            pltpu.SemaphoreType.DMA((NB,)),
            pltpu.SemaphoreType.DMA((B,)),
        ],
        compiler_params=pltpu.CompilerParams(
            vmem_limit_bytes=96 * 1024 * 1024,
            disable_bounds_checks=True,
        ),
    )(x, k_cache, v_cache, wq, wo.T)
    return out
```

```python
import functools

import jax
import jax.numpy as jnp
import jax.experimental.pallas as pl
import jax.experimental.pallas.tpu as pltpu

HQ = 16
DH = 256
NB = 8
LEAD = 1
NSB = LEAD + 1
U = 2
CK = 512
SUB = 64
WSUB = 32
LA = 4
NODMA = 0
BLK = 0
LIGHT = 0
G = 2
GW = 1
assert U % GW == 0
assert U % NSB == 0


def _divmod_pow2(t, n):
    assert n & (n - 1) == 0
    if isinstance(t, int):
        return t // n, t % n
    sh = n.bit_length() - 1
    return jax.lax.shift_right_logical(t, sh), jax.lax.bitwise_and(t, n - 1)


def _kernel(x_hbm, k_hbm, v_hbm, wq_hbm, wo_hbm, out_hbm,
            xbuf, wqbuf, wobuf, kvbuf, acc, obuf, *rest,
            B, Sq, Hkv, Sk, D, rep, scale):
    kbuf = kvbuf.at[0]
    vbuf = kvbuf.at[1]
    sbufs = rest[:NSB]
    mbufs = rest[NSB:2 * NSB]
    xsem, wqsem, wosem, ksem, vsem, osem = rest[2 * NSB:]
    T = B * Hkv
    W = rep * DH
    M = rep * Sq
    NC = Sk // CK
    NS = CK // SUB
    f32 = jnp.float32
    bf16 = jnp.bfloat16

    def hb(t):
        return _divmod_pow2(t, B)

    def slot_of(t):
        return _divmod_pow2(t, NB)[1]

    def when(cond, fn):
        if isinstance(cond, bool):
            if cond:
                fn()
        else:
            pl.when(cond)(fn)

    def land(a, b):
        if isinstance(a, bool) and isinstance(b, bool):
            return a and b
        return jnp.logical_and(a, b)

    def blk_copy(hbm, buf, sem, t, r0, nrows):
        h, b = hb(t)
        slot = slot_of(t)
        return pltpu.make_async_copy(hbm.at[b, h, :, pl.ds(r0, nrows)], buf.at[slot, :, pl.ds(r0, nrows)],
                                     sem.at[slot])

    def w_copy(hbm, buf, sem, h, r0, nrows):
        if not isinstance(r0, int):
            r0 = pl.multiple_of(r0, 8)
        return pltpu.make_async_copy(hbm.at[pl.ds(r0, nrows), pl.ds(h * W, W)], buf.at[h, pl.ds(r0, nrows)],
                                     sem.at[h])

    def issue_d(p, c):
        tk = p + LEAD
        tv = p
        static = isinstance(p, int)
        k_ok = tk < T
        v_ok = (0 <= tv < T) if static else tv < T
        if static and not k_ok and not v_ok:
            return
        hk, bk = hb(tk)
        hv, bv = hb(max(tv, 0) if static else tv)
        WP = D // B
        pieces = [(0, WSUB), (WSUB, WP - WSUB)] if WP > WSUB else [(0, WP)]
        if c == 0:
            if static and tk == 0:
                for i, r0 in enumerate(range(0, D, WSUB)):
                    w_copy(wq_hbm, wqbuf, wqsem, 0, r0, WSUB).start(priority=i % 2)
            for i, (o_, n_) in enumerate(pieces):
                when(land(k_ok, hk + 1 < Hkv),
                     lambda: w_copy(wq_hbm, wqbuf, wqsem, hk + 1, bk * WP + o_, n_).start(priority=i % 2))
        if c == NC - 1:
            if static and tv == 0:
                for i, r0 in enumerate(range(0, D, WSUB)):
                    w_copy(wo_hbm, wobuf, wosem, 0, r0, WSUB).start(priority=i % 2)
            for i, (o_, n_) in enumerate(pieces):
                when(land(v_ok, hv + 1 < Hkv),
                     lambda: w_copy(wo_hbm, wobuf, wosem, hv + 1, bv * WP + o_, n_).start(priority=(i + 1) % 2))
        single = static and not (k_ok and v_ok)
        if NODMA == 1:
            return
        for j in range(NS):
            r0 = (c * CK + j * SUB) // G
            when(k_ok, lambda: blk_copy(k_hbm, kbuf, ksem, tk, r0, SUB // G).start(
                priority=(j % 2) if (single or BLK) else 0))
            if NODMA == 2:
                continue
            when(v_ok, lambda: blk_copy(v_hbm, vbuf, vsem, tv, r0, SUB // G).start(
                priority=((j + 1) % 2) if (single or BLK) else 1))

    def wait_wq(t):
        h, b = hb(t)
        when(b == 0, lambda: w_copy(wq_hbm, wqbuf, wqsem, h, 0, D).wait())

    def wait_wo(t):
        h, b = hb(t)
        when(b == 0, lambda: w_copy(wo_hbm, wobuf, wosem, h, 0, D).wait())

    def wait_k(t):
        if NODMA != 1:
            blk_copy(k_hbm, kbuf, ksem, t, 0, Sk // G).wait()

    def wait_v(t):
        if not NODMA:
            blk_copy(v_hbm, vbuf, vsem, t, 0, Sk // G).wait()

    def x_copy(b):
        return pltpu.make_async_copy(x_hbm.at[b], xbuf.at[b], xsem.at[b])

    def o_copy(b):
        return pltpu.make_async_copy(obuf.at[b], out_hbm.at[b], osem.at[b])

    def q_proj(t):
        h, b = hb(t)
        q = jnp.dot(xbuf[b], wqbuf[h], preferred_element_type=f32)
        qb = (q.astype(bf16) * scale).astype(bf16)
        return jnp.concatenate([qb[:, r * DH:(r + 1) * DH] for r in range(rep)], axis=0)

    def a_chunk(t, sb, q2, c, mrun):
        slot = slot_of(t)
        g, r = divmod(c * CK, Sk // G)
        kc = kbuf[slot, g, r:r + CK, :]
        s = jax.lax.dot_general(q2, kc, (((1,), (1,)), ((), ())), preferred_element_type=f32)
        sbufs[sb][:, c * CK:(c + 1) * CK] = s
        for j in range(CK // 128):
            sj = s[:, j * 128:(j + 1) * 128]
            mrun = sj if mrun is None else jnp.maximum(mrun, sj)
        return mrun

    def a_fin(sb, mrun):
        m = jnp.max(mrun, axis=-1, keepdims=True)
        mbufs[sb][...] = jnp.broadcast_to(m, (M, 128))

    def b_chunk(t, sb, m128, c, lrun, o):
        slot = slot_of(t)
        ps = []
        for j in range(CK // 128):
            sj = sbufs[sb][:, c * CK + j * 128:c * CK + (j + 1) * 128]
            pj = jnp.exp(sj - m128)
            lrun = pj if lrun is None else lrun + pj
            ps.append(pj.astype(bf16))
        p = jnp.concatenate(ps, axis=1)
        g, r = divmod(c * CK, Sk // G)
        vc = vbuf[slot, g, r:r + CK, :]
        oc = jnp.dot(p, vc, preferred_element_type=f32)
        o = oc if o is None else o + oc
        return lrun, o

    def b_fin(t, lrun, o):
        h, b = hb(t)
        l = jnp.sum(lrun, axis=-1, keepdims=True)
        o = (o / l).astype(bf16)
        o2 = jnp.concatenate([o[r * Sq:(r + 1) * Sq, :] for r in range(rep)], axis=1)
        contrib = jax.lax.dot_general(o2, wobuf[h], (((1,), (1,)), ((), ())),
                                      preferred_element_type=f32)
        new = acc[b] + contrib
        acc[b] = new
        obuf[b] = new.astype(obuf.dtype)

    def issue_for(t, c):
        q = c + LA
        issue_d(t + GW + q // NC, q % NC)

    def stage(t, tmod, do_a, do_b):
        sa = (tmod + LEAD) % NSB
        sb = tmod % NSB
        if LIGHT < 0 and not isinstance(t, int):
            for c in range(NC):
                issue_for(t, c)
            return
        if do_a:
            q2 = q_proj(t + LEAD)
        if do_b:
            m128 = mbufs[sb][...]
        mrun = None
        lrun = None
        o = None
        for c in range(NC):
            issue_for(t, c)
            if LIGHT > 0 and c >= LIGHT and not isinstance(t, int):
                continue
            if do_b:
                lrun, o = b_chunk(t, sb, m128, c, lrun, o)
            if do_a:
                mrun = a_chunk(t + LEAD, sa, q2, c, mrun)
        if do_a:
            a_fin(sa, mrun)
        if do_b:
            b_fin(t, lrun, o)

    def group(t0, n, tmod0):
        flags = []
        for j in range(n):
            t = t0 + j
            do_a = (t + LEAD < T) if isinstance(t, int) else True
            do_b = (t >= 0) if isinstance(t, int) else True
            flags.append((do_a, do_b))
            if do_a:
                wait_wq(t + LEAD)
                wait_k(t + LEAD)
            if do_b:
                wait_v(t)
                wait_wo(t)
        for j in range(n):
            stage(t0 + j, (tmod0 + j) % NSB, *flags[j])
        for j in range(n):
            if flags[j][1]:
                h, b = hb(t0 + j)
                when(h == Hkv - 1, lambda: o_copy(b).start())

    x_copy(0).start(priority=1)
    for c in range(NC):
        issue_d(-LEAD, c)
    for b in range(1, B):
        x_copy(b).start(priority=b % 2)
    acc[...] = jnp.zeros(acc.shape, acc.dtype)
    for g in range(NC, NC * GW + LA):
        issue_d(-LEAD + g // NC, g % NC)
    for b in range(B):
        x_copy(b).wait()
    for t in range(-LEAD, 0):
        group(t, 1, t % NSB)

    n_full = T - LEAD
    n_loop = n_full // U

    def body(u, carry):
        for g in range(U // GW):
            group(u * U + g * GW, GW, (g * GW) % NSB)
        return carry

    jax.lax.fori_loop(0, n_loop, body, 0)

    for t in range(n_loop * U, T):
        group(t, 1, t % NSB)
    for b in range(B):
        o_copy(b).wait()


@jax.jit
def pallas_standalone__gqa_block_cached__near_ridge_kernel(
    x: jax.Array,
    k_cache: jax.Array,
    v_cache: jax.Array,
    wq: jax.Array,
    wo: jax.Array,
):
    B, Sq, D = x.shape
    _, Hkv, Sk, Dh = k_cache.shape
    assert Dh == DH
    rep = HQ // Hkv
    W = rep * Dh
    M = rep * Sq
    scale = float(Dh) ** -0.5

    kern = functools.partial(_kernel, B=B, Sq=Sq, Hkv=Hkv, Sk=Sk, D=D, rep=rep, scale=scale)
    any_spec = pl.BlockSpec(memory_space=pl.ANY)
    out = pl.pallas_call(
        kern,
        in_specs=[any_spec] * 5,
        out_specs=any_spec,
        out_shape=jax.ShapeDtypeStruct((B, Sq, D), x.dtype),
        scratch_shapes=[
            pltpu.VMEM((B, Sq, D), jnp.bfloat16),
            pltpu.VMEM((Hkv, D, W), jnp.bfloat16),
            pltpu.VMEM((Hkv, D, W), jnp.bfloat16),
            pltpu.VMEM((2, NB, G, Sk // G, Dh), jnp.bfloat16),
            pltpu.VMEM((B, Sq, D), jnp.float32),
            pltpu.VMEM((B, Sq, D), jnp.bfloat16),
        ] + [pltpu.VMEM((M, Sk), jnp.float32)] * NSB + [pltpu.VMEM((M, 128), jnp.float32)] * NSB + [
            pltpu.SemaphoreType.DMA((B,)),
            pltpu.SemaphoreType.DMA((Hkv,)),
            pltpu.SemaphoreType.DMA((Hkv,)),
            pltpu.SemaphoreType.DMA((NB,)),
            pltpu.SemaphoreType.DMA((NB,)),
            pltpu.SemaphoreType.DMA((B,)),
        ],
        compiler_params=pltpu.CompilerParams(
            vmem_limit_bytes=96 * 1024 * 1024,
            disable_bounds_checks=True,
        ),
    )(x, k_cache.reshape(B, Hkv, G, Sk // G, Dh), v_cache.reshape(B, Hkv, G, Sk // G, Dh), wq, wo.T)
    return out
```

```python
import functools

import jax
import jax.numpy as jnp
import jax.experimental.pallas as pl
import jax.experimental.pallas.tpu as pltpu

HQ = 16
DH = 256
NB = 8
CK = 512
G = 2
SUB = 64
WSUB = 32
AHEAD = 2
SEQ = ("i0", "i1", "a0", "b0", "a1", "b1", "i2", "i3", "a2", "b2", "b3", "a3")


def _divmod_pow2(t, n):
    assert n & (n - 1) == 0
    if isinstance(t, int):
        return t // n, t % n
    sh = n.bit_length() - 1
    return jax.lax.shift_right_logical(t, sh), jax.lax.bitwise_and(t, n - 1)


def _when(cond, fn):
    if isinstance(cond, bool):
        if cond:
            fn()
    else:
        pl.when(cond)(fn)


def _and(a, b):
    if isinstance(a, bool) and isinstance(b, bool):
        return a and b
    return jnp.logical_and(a, b)


def _kernel(x_hbm, k_hbm, v_hbm, wq_hbm, wo_hbm, out_hbm,
            xbuf, wqbuf, wobuf, kvbuf, acc, obuf, s0, s1, m0, m1,
            xsem, wqsem, wosem, ksem, vsem, osem,
            *, B, Sq, Hkv, Sk, D, rep, scale):
    kbuf = kvbuf.at[0]
    vbuf = kvbuf.at[1]
    sbufs = (s0, s1)
    mbufs = (m0, m1)
    T = B * Hkv
    W = rep * DH
    M = rep * Sq
    NC = Sk // CK
    NS = CK // SUB
    L = Sk // G
    WP = D // B
    f32 = jnp.float32
    bf16 = jnp.bfloat16

    def hb(t):
        return _divmod_pow2(t, B)

    def slot_of(t):
        return _divmod_pow2(t, NB)[1]

    def blk_copy(hbm, buf, sem, t, r0, nrows):
        h, b = hb(t)
        slot = slot_of(t)
        return pltpu.make_async_copy(hbm.at[b, h, :, pl.ds(r0, nrows)],
                                     buf.at[slot, :, pl.ds(r0, nrows)], sem.at[slot])

    def w_copy(hbm, buf, sem, h, r0, nrows):
        if not isinstance(r0, int):
            r0 = pl.multiple_of(r0, 8)
        return pltpu.make_async_copy(hbm.at[pl.ds(r0, nrows), pl.ds(h * W, W)],
                                     buf.at[h, pl.ds(r0, nrows)], sem.at[h])

    def x_copy(b):
        return pltpu.make_async_copy(x_hbm.at[b], xbuf.at[b], xsem.at[b])

    def o_copy(b):
        return pltpu.make_async_copy(obuf.at[b], out_hbm.at[b], osem.at[b])

    w_pieces = [(0, WSUB), (WSUB, WP - WSUB)] if WP > WSUB else [(0, WP)]

    def issue_d(p, c):
        tk = p + 1
        tv = p
        static = isinstance(p, int)
        k_ok = tk < T
        v_ok = (0 <= tv < T) if static else tv < T
        if static and not k_ok and not v_ok:
            return
        hk, bk = hb(tk)
        hv, bv = hb(max(tv, 0) if static else tv)
        if c == 0:
            if static and tk == 0:
                for i, r0 in enumerate(range(0, D, WSUB)):
                    w_copy(wq_hbm, wqbuf, wqsem, 0, r0, WSUB).start(priority=i % 2)
            for i, (off, n) in enumerate(w_pieces):
                _when(_and(k_ok, hk + 1 < Hkv),
                      lambda: w_copy(wq_hbm, wqbuf, wqsem, hk + 1, bk * WP + off, n).start(priority=i % 2))
        if c == NC - 1:
            if static and tv == 0:
                for i, r0 in enumerate(range(0, D, WSUB)):
                    w_copy(wo_hbm, wobuf, wosem, 0, r0, WSUB).start(priority=i % 2)
            for i, (off, n) in enumerate(w_pieces):
                _when(_and(v_ok, hv + 1 < Hkv),
                      lambda: w_copy(wo_hbm, wobuf, wosem, hv + 1, bv * WP + off, n).start(priority=(i + 1) % 2))
        single = static and not (k_ok and v_ok)
        for j in range(NS):
            r0 = (c * CK + j * SUB) // G
            _when(k_ok, lambda: blk_copy(k_hbm, kbuf, ksem, tk, r0, SUB // G).start(
                priority=(j % 2) if single else 0))
            _when(v_ok, lambda: blk_copy(v_hbm, vbuf, vsem, tv, r0, SUB // G).start(
                priority=((j + 1) % 2) if single else 1))

    def wait_a_inputs(t):
        h, b = hb(t)
        _when(b == 0, lambda: w_copy(wq_hbm, wqbuf, wqsem, h, 0, D).wait())
        blk_copy(k_hbm, kbuf, ksem, t, 0, L).wait()

    def wait_b_inputs(t):
        h, b = hb(t)
        blk_copy(v_hbm, vbuf, vsem, t, 0, L).wait()
        _when(b == 0, lambda: w_copy(wo_hbm, wobuf, wosem, h, 0, D).wait())

    def q_proj(t):
        h, b = hb(t)
        q = jnp.dot(xbuf[b], wqbuf[h], preferred_element_type=f32)
        qb = (q * scale).astype(bf16)
        return jnp.concatenate([qb[:, r * DH:(r + 1) * DH] for r in range(rep)], axis=0)

    def a_chunk(t, par, q2, c, mrun):
        g, r = divmod(c * CK, L)
        kc = kbuf[slot_of(t), g, r:r + CK, :]
        s = jax.lax.dot_general(q2, kc, (((1,), (1,)), ((), ())), preferred_element_type=f32)
        sbufs[par][:, c * CK:(c + 1) * CK] = s
        for j in range(CK // 128):
            sj = s[:, j * 128:(j + 1) * 128]
            mrun = sj if mrun is None else jnp.maximum(mrun, sj)
        return mrun

    def a_fin(par, mrun):
        m = jnp.max(mrun, axis=-1, keepdims=True)
        mbufs[par][...] = jnp.broadcast_to(m, (M, 128))

    def b_chunk(t, par, m128, c, lrun, o):
        ps = []
        for j in range(CK // 128):
            lo = c * CK + j * 128
            pj = jnp.exp(sbufs[par][:, lo:lo + 128] - m128)
            lrun = pj if lrun is None else lrun + pj
            ps.append(pj.astype(bf16))
        p = jnp.concatenate(ps, axis=1)
        g, r = divmod(c * CK, L)
        vc = vbuf[slot_of(t), g, r:r + CK, :]
        oc = jnp.dot(p, vc, preferred_element_type=f32)
        return lrun, (oc if o is None else o + oc)

    def b_fin(t, lrun, o):
        h, b = hb(t)
        l = jnp.sum(lrun, axis=-1, keepdims=True)
        o = (o / l).astype(bf16)
        o2 = jnp.concatenate([o[r * Sq:(r + 1) * Sq, :] for r in range(rep)], axis=1)
        contrib = jax.lax.dot_general(o2, wobuf[h], (((1,), (1,)), ((), ())),
                                      preferred_element_type=f32)
        new = acc[b] + contrib
        acc[b] = new
        obuf[b] = new.astype(obuf.dtype)

    def stage(t, par):
        static = isinstance(t, int)
        do_a = (t + 1 < T) if static else True
        do_b = (t >= 0) if static else True
        if do_a:
            wait_a_inputs(t + 1)
        if do_b:
            wait_b_inputs(t)
        if do_a:
            q2 = q_proj(t + 1)
        if do_b:
            m128 = mbufs[par][...]
        mrun = lrun = o = None
        for tok in SEQ:
            kind, c = tok[0], int(tok[1:])
            if kind == "i":
                issue_d(t + AHEAD, c)
            elif kind == "b" and do_b:
                lrun, o = b_chunk(t, par, m128, c, lrun, o)
            elif kind == "a" and do_a:
                mrun = a_chunk(t + 1, 1 - par, q2, c, mrun)
        if do_a:
            a_fin(1 - par, mrun)
        if do_b:
            b_fin(t, lrun, o)
            h, b = hb(t)
            _when(h == Hkv - 1, lambda: o_copy(b).start())

    x_copy(0).start(priority=1)
    for c in range(NC):
        issue_d(-1, c)
    for b in range(1, B):
        x_copy(b).start(priority=b % 2)
    acc[...] = jnp.zeros(acc.shape, acc.dtype)
    for p in range(0, AHEAD - 1):
        for c in range(NC):
            issue_d(p, c)
    for b in range(B):
        x_copy(b).wait()
    stage(-1, 1)

    n_loop = (T - 1) // 2

    def body(u, carry):
        stage(2 * u, 0)
        stage(2 * u + 1, 1)
        return carry

    jax.lax.fori_loop(0, n_loop, body, 0)

    for t in range(2 * n_loop, T):
        stage(t, t % 2)
    for b in range(B):
        o_copy(b).wait()


@jax.jit
def pallas_standalone__gqa_block_cached__near_ridge_kernel(
    x: jax.Array,
    k_cache: jax.Array,
    v_cache: jax.Array,
    wq: jax.Array,
    wo: jax.Array,
):
    B, Sq, D = x.shape
    _, Hkv, Sk, Dh = k_cache.shape
    assert Dh == DH and Sk // CK == 4 and D % (8 * B) == 0 and D % WSUB == 0
    rep = HQ // Hkv
    W = rep * Dh
    M = rep * Sq
    scale = float(Dh) ** -0.5

    kern = functools.partial(_kernel, B=B, Sq=Sq, Hkv=Hkv, Sk=Sk, D=D, rep=rep, scale=scale)
    any_spec = pl.BlockSpec(memory_space=pl.ANY)
    return pl.pallas_call(
        kern,
        in_specs=[any_spec] * 5,
        out_specs=any_spec,
        out_shape=jax.ShapeDtypeStruct((B, Sq, D), x.dtype),
        scratch_shapes=[
            pltpu.VMEM((B, Sq, D), jnp.bfloat16),
            pltpu.VMEM((Hkv, D, W), jnp.bfloat16),
            pltpu.VMEM((Hkv, D, W), jnp.bfloat16),
            pltpu.VMEM((2, NB, G, Sk // G, Dh), jnp.bfloat16),
            pltpu.VMEM((B, Sq, D), jnp.float32),
            pltpu.VMEM((B, Sq, D), jnp.bfloat16),
            pltpu.VMEM((M, Sk), jnp.float32),
            pltpu.VMEM((M, Sk), jnp.float32),
            pltpu.VMEM((M, 128), jnp.float32),
            pltpu.VMEM((M, 128), jnp.float32),
            pltpu.SemaphoreType.DMA((B,)),
            pltpu.SemaphoreType.DMA((Hkv,)),
            pltpu.SemaphoreType.DMA((Hkv,)),
            pltpu.SemaphoreType.DMA((NB,)),
            pltpu.SemaphoreType.DMA((NB,)),
            pltpu.SemaphoreType.DMA((B,)),
        ],
        compiler_params=pltpu.CompilerParams(
            vmem_limit_bytes=96 * 1024 * 1024,
            disable_bounds_checks=True,
        ),
    )(x, k_cache.reshape(B, Hkv, G, Sk // G, Dh), v_cache.reshape(B, Hkv, G, Sk // G, Dh), wq, wo.T)
```

```python
import functools

import jax
import jax.numpy as jnp
import jax.experimental.pallas as pl
import jax.experimental.pallas.tpu as pltpu

HQ = 16
DH = 256
NB = 4
CK = 512
R = 16
WSUB = 16
NQ = 4
SEQ = (("i0", "i1", "b0", "a0", "b1", "a1", "i2", "i3", "b2", "a2", "b3", "a3"),
       ("a0", "i0", "i1", "b0", "b2", "a2", "i2", "i3", "b1", "a1", "b3", "a3"))


def _divmod_pow2(t, n):
    assert n & (n - 1) == 0
    if isinstance(t, int):
        return t // n, t % n
    sh = n.bit_length() - 1
    return jax.lax.shift_right_logical(t, sh), jax.lax.bitwise_and(t, n - 1)


def _when(cond, fn):
    if isinstance(cond, bool):
        if cond:
            fn()
    else:
        pl.when(cond)(fn)


def _and(a, b):
    if isinstance(a, bool) and isinstance(b, bool):
        return a and b
    return jnp.logical_and(a, b)


def _kernel(x_hbm, k_hbm, v_hbm, wq_hbm, wo_hbm, out_hbm,
            xbuf, wqbuf, wobuf, kvbuf, acc, obuf, qbuf, mpart, lpart, opart,
            s00, s01, s10, s11, m00, m01, m10, m11,
            xsem, wqsem, wosem, ksem, vsem, osem,
            *, B, Sq, Hkv, Sk, D, rep, scale):
    kbuf = kvbuf.at[0]
    vbuf = kvbuf.at[1]
    sbufs = ((s00, s01), (s10, s11))
    mbufs = ((m00, m01), (m10, m11))
    HP = Hkv // 2
    NU = B * HP
    W = rep * DH
    W2 = 2 * W
    M = rep * Sq
    L = Sk // 2
    NR = CK // R
    WPB = D // B
    f32 = jnp.float32
    bf16 = jnp.bfloat16

    def bh(u):
        hp, b = _divmod_pow2(u, B)
        return b, hp

    def slot_of(u):
        return _divmod_pow2(u, NB)[1]

    def blk_copy(hbm, buf, sem, u, s, r0, nrows):
        b, hp = bh(u)
        slot = slot_of(u)
        return pltpu.make_async_copy(hbm.at[b * HP + hp, :, pl.ds(r0, nrows)],
                                     buf.at[slot, :, pl.ds(r0, nrows)], sem.at[2 * slot + s])

    def w_copy(hbm, buf, sem, hp, r0, nrows):
        if not isinstance(r0, int):
            r0 = pl.multiple_of(r0, 8)
        return pltpu.make_async_copy(hbm.at[pl.ds(r0, nrows), pl.ds(hp * W2, W2)],
                                     buf.at[hp, pl.ds(r0, nrows)], sem.at[hp])

    def x_copy(b):
        return pltpu.make_async_copy(x_hbm.at[b], xbuf.at[b], xsem.at[b])

    def o_copy(b):
        return pltpu.make_async_copy(obuf.at[b], out_hbm.at[b], osem.at[b])

    w_pieces = [(off, min(WSUB, WPB - off)) for off in range(0, WPB, WSUB)]
    n_half = (len(w_pieces) + 1) // 2
    w_pieces = (w_pieces[:n_half], w_pieces[n_half:])

    def issue_d(u, s, c):
        uk = u + 1
        uv = u
        static = isinstance(u, int)
        k_ok = uk < NU
        v_ok = (0 <= uv < NU) if static else uv < NU
        if static and not k_ok and not v_ok:
            return
        bk, hk = bh(uk)
        bv, hv = bh(max(uv, 0) if static else uv)
        if c == 0:
            if static and uk == 0 and s == 0:
                for i, r0 in enumerate(range(0, D, WSUB)):
                    w_copy(wq_hbm, wqbuf, wqsem, 0, r0, WSUB).start(priority=i % 2)
            for i, (off, n) in enumerate(w_pieces[s]):
                _when(_and(k_ok, hk + 1 < HP),
                      lambda: w_copy(wq_hbm, wqbuf, wqsem, hk + 1, bk * WPB + off, n).start(priority=i % 2))
        if c == NQ - 1:
            if static and uv == 0 and s == 0:
                for i, r0 in enumerate(range(0, D, WSUB)):
                    w_copy(wo_hbm, wobuf, wosem, 0, r0, WSUB).start(priority=i % 2)
            for i, (off, n) in enumerate(w_pieces[s]):
                _when(_and(v_ok, hv + 1 < HP),
                      lambda: w_copy(wo_hbm, wobuf, wosem, hv + 1, bv * WPB + off, n).start(priority=(i + 1) % 2))
        single = static and not (k_ok and v_ok)
        for j in range(NR // NQ):
            r0 = s * CK + (c * (NR // NQ) + j) * R
            _when(k_ok, lambda: blk_copy(k_hbm, kbuf, ksem, uk, s, r0, R).start(
                priority=(j % 2) if single else 0))
            _when(v_ok, lambda: blk_copy(v_hbm, vbuf, vsem, uv, s, r0, R).start(
                priority=((j + 1) % 2) if single else 1))

    def wait_a_inputs(u, s):
        if s == 0:
            b, hp = bh(u)
            _when(b == 0, lambda: w_copy(wq_hbm, wqbuf, wqsem, hp, 0, D).wait())
        blk_copy(k_hbm, kbuf, ksem, u, s, s * CK, CK).wait()

    def wait_b_inputs(u, s):
        blk_copy(v_hbm, vbuf, vsem, u, s, s * CK, CK).wait()
        if s == 1:
            b, hp = bh(u)
            _when(b == 0, lambda: w_copy(wo_hbm, wobuf, wosem, hp, 0, D).wait())

    def q_proj(u):
        b, hp = bh(u)
        q = jnp.dot(xbuf[b], wqbuf[hp], preferred_element_type=f32)
        qb = (q * scale).astype(bf16)
        qs = []
        for e in range(2):
            qe = jnp.concatenate([qb[:, e * W + r * DH:e * W + (r + 1) * DH] for r in range(rep)], axis=0)
            qbuf[e] = qe
            qs.append(qe)
        return qs

    def a_chunk(u, s, par, qs, c, mrun):
        e, g = divmod(c, 2)
        kc = kbuf[slot_of(u), c, s * CK:(s + 1) * CK, :]
        sc = jax.lax.dot_general(qs[e], kc, (((1,), (1,)), ((), ())), preferred_element_type=f32)
        lo = g * L + s * CK
        sbufs[par][e][:, lo:lo + CK] = sc
        mr = mrun[e]
        for j in range(CK // 128):
            sj = sc[:, j * 128:(j + 1) * 128]
            mr = sj if mr is None else jnp.maximum(mr, sj)
        mrun[e] = mr

    def b_chunk(u, s, par, m128, c, lrun, o):
        e, g = divmod(c, 2)
        ps = []
        lr = lrun[e]
        for j in range(CK // 128):
            lo = g * L + s * CK + j * 128
            pj = jnp.exp(sbufs[par][e][:, lo:lo + 128] - m128[e])
            lr = pj if lr is None else lr + pj
            ps.append(pj.astype(bf16))
        lrun[e] = lr
        p = jnp.concatenate(ps, axis=1)
        vc = vbuf[slot_of(u), c, s * CK:(s + 1) * CK, :]
        oc = jnp.dot(p, vc, preferred_element_type=f32)
        o[e] = oc if o[e] is None else o[e] + oc

    def b_fin(u, lrun, o):
        b, hp = bh(u)
        cols = []
        for e in range(2):
            l = jnp.sum(lrun[e], axis=-1, keepdims=True)
            oe = (o[e] / l).astype(bf16)
            cols += [oe[r * Sq:(r + 1) * Sq, :] for r in range(rep)]
        o2 = jnp.concatenate(cols, axis=1)
        contrib = jax.lax.dot_general(o2, wobuf[hp], (((1,), (1,)), ((), ())),
                                      preferred_element_type=f32)
        new = acc[b] + contrib
        acc[b] = new
        obuf[b] = new.astype(obuf.dtype)
        _when(hp == HP - 1, lambda: o_copy(b).start())

    def stage(u, s, par):
        static = isinstance(u, int)
        do_a = (u + 1 < NU) if static else True
        do_b = (u >= 0) if static else True
        if do_a:
            wait_a_inputs(u + 1, s)
        if do_b:
            wait_b_inputs(u, s)
        if do_a:
            if s == 0:
                qs = q_proj(u + 1)
                mrun = [None, None]
            else:
                qs = [qbuf[0], qbuf[1]]
                mrun = [mpart[0], mpart[1]]
        if do_b:
            m128 = [mbufs[par][0][...], mbufs[par][1][...]]
            if s == 0:
                lrun = [None, None]
                o = [None, None]
            else:
                lrun = [lpart[0], lpart[1]]
                o = [opart[0], opart[1]]
        for tok in SEQ[s]:
            kind, c = tok[0], int(tok[1:])
            if kind == "i":
                issue_d(u + 1, s, c)
            elif kind == "b" and do_b:
                b_chunk(u, s, par, m128, c, lrun, o)
            elif kind == "a" and do_a:
                a_chunk(u + 1, s, 1 - par, qs, c, mrun)
        if do_a:
            for e in range(2):
                if s == 0:
                    mpart[e] = mrun[e]
                else:
                    m = jnp.max(mrun[e], axis=-1, keepdims=True)
                    mbufs[1 - par][e][...] = jnp.broadcast_to(m, (M, 128))
        if do_b:
            if s == 0:
                for e in range(2):
                    lpart[e] = lrun[e]
                    opart[e] = o[e]
            else:
                b_fin(u, lrun, o)

    def last_stage(u, par):
        wait_b_inputs(u, 0)
        wait_b_inputs(u, 1)
        m128 = [mbufs[par][0][...], mbufs[par][1][...]]
        lrun = [None, None]
        o = [None, None]
        for s in range(2):
            for c in (0, 2, 1, 3):
                b_chunk(u, s, par, m128, c, lrun, o)
        b_fin(u, lrun, o)

    x_copy(0).start(priority=1)
    for c in range(NQ):
        issue_d(-1, 0, c)
    for b in range(1, B):
        x_copy(b).start(priority=b % 2)
    acc[...] = jnp.zeros(acc.shape, acc.dtype)
    for c in range(NQ):
        issue_d(-1, 1, c)
    for b in range(B):
        x_copy(b).wait()
    n_static = (NU - 1) % 2
    for u in range(-1, n_static):
        stage(u, 0, u % 2)
        stage(u, 1, u % 2)

    def body(i, carry):
        u = n_static + 2 * i
        for d in range(2):
            stage(u + d, 0, (n_static + d) % 2)
            stage(u + d, 1, (n_static + d) % 2)
        return carry

    jax.lax.fori_loop(0, (NU - 1 - n_static) // 2, body, 0)

    last_stage(NU - 1, (NU - 1) % 2)
    for b in range(B):
        o_copy(b).wait()


@jax.jit
def pallas_standalone__gqa_block_cached__near_ridge_kernel(
    x: jax.Array,
    k_cache: jax.Array,
    v_cache: jax.Array,
    wq: jax.Array,
    wo: jax.Array,
):
    B, Sq, D = x.shape
    _, Hkv, Sk, Dh = k_cache.shape
    assert Dh == DH and Sk == 4 * CK and Hkv % 2 == 0 and D % WSUB == 0 and D % (8 * B) == 0
    rep = HQ // Hkv
    W = rep * Dh
    M = rep * Sq
    HP = Hkv // 2
    NU = B * HP
    scale = float(Dh) ** -0.5

    kern = functools.partial(_kernel, B=B, Sq=Sq, Hkv=Hkv, Sk=Sk, D=D, rep=rep, scale=scale)
    any_spec = pl.BlockSpec(memory_space=pl.ANY)
    f32, bf16 = jnp.float32, jnp.bfloat16
    return pl.pallas_call(
        kern,
        in_specs=[any_spec] * 5,
        out_specs=any_spec,
        out_shape=jax.ShapeDtypeStruct((B, Sq, D), x.dtype),
        scratch_shapes=[
            pltpu.VMEM((B, Sq, D), bf16),
            pltpu.VMEM((HP, D, 2 * W), bf16),
            pltpu.VMEM((HP, D, 2 * W), bf16),
            pltpu.VMEM((2, NB, 4, Sk // 2, Dh), bf16),
            pltpu.VMEM((B, Sq, D), f32),
            pltpu.VMEM((B, Sq, D), bf16),
            pltpu.VMEM((2, M, Dh), bf16),
            pltpu.VMEM((2, M, 128), f32),
            pltpu.VMEM((2, M, 128), f32),
            pltpu.VMEM((2, M, Dh), f32),
        ] + [pltpu.VMEM((M, Sk), f32)] * 4
          + [pltpu.VMEM((M, 128), f32)] * 4
          + [
            pltpu.SemaphoreType.DMA((B,)),
            pltpu.SemaphoreType.DMA((HP,)),
            pltpu.SemaphoreType.DMA((HP,)),
            pltpu.SemaphoreType.DMA((2 * NB,)),
            pltpu.SemaphoreType.DMA((2 * NB,)),
            pltpu.SemaphoreType.DMA((B,)),
        ],
        compiler_params=pltpu.CompilerParams(
            vmem_limit_bytes=96 * 1024 * 1024,
            disable_bounds_checks=True,
        ),
    )(x, k_cache.reshape(NU, 4, Sk // 2, Dh), v_cache.reshape(NU, 4, Sk // 2, Dh), wq, wo.T)
```

```python
import functools

import jax
import jax.numpy as jnp
import jax.experimental.pallas as pl
import jax.experimental.pallas.tpu as pltpu

HQ = 16
DH = 256
NB = 4
CK = 512
R = 16
WSUB = 16
NQ = 4
SEQ = (("i0", "i1", "b0", "a0", "b1", "a1", "i2", "i3", "b2", "a2", "b3", "a3"),
       ("a0", "i0", "i1", "b0", "b2", "a2", "i2", "i3", "b1", "a1", "b3", "a3"))


def _divmod_pow2(t, n):
    assert n & (n - 1) == 0
    if isinstance(t, int):
        return t // n, t % n
    sh = n.bit_length() - 1
    return jax.lax.shift_right_logical(t, sh), jax.lax.bitwise_and(t, n - 1)


def _when(cond, fn):
    if isinstance(cond, bool):
        if cond:
            fn()
    else:
        pl.when(cond)(fn)


def _and(a, b):
    if isinstance(a, bool) and isinstance(b, bool):
        return a and b
    return jnp.logical_and(a, b)


def _kernel(x_hbm, k_hbm, v_hbm, wq_hbm, wo_hbm, out_hbm,
            xbuf, wqbuf, wobuf, kvbuf, acc, obuf, qbuf, mpart, lpart, opart,
            s00, s01, s10, s11, m00, m01, m10, m11,
            xsem, wqsem, wosem, ksem, vsem, osem,
            *, B, Sq, Hkv, Sk, D, rep, scale):
    kbuf = kvbuf.at[0]
    vbuf = kvbuf.at[1]
    sbufs = ((s00, s01), (s10, s11))
    mbufs = ((m00, m01), (m10, m11))
    HP = Hkv // 2
    NU = B * HP
    W = rep * DH
    W2 = 2 * W
    M = rep * Sq
    L = Sk // 2
    NR = CK // R
    WPB = D // B
    f32 = jnp.float32
    bf16 = jnp.bfloat16

    def bh(u):
        hp, b = _divmod_pow2(u, B)
        return b, hp

    def slot_of(u):
        return _divmod_pow2(u, NB)[1]

    def blk_copy(hbm, buf, sem, u, s, r0, nrows):
        b, hp = bh(u)
        slot = slot_of(u)
        return pltpu.make_async_copy(hbm.at[b * HP + hp, :, pl.ds(r0, nrows)],
                                     buf.at[slot, :, pl.ds(r0, nrows)], sem.at[2 * slot + s])

    def w_copy(hbm, buf, sem, hp, r0, nrows):
        if not isinstance(r0, int):
            r0 = pl.multiple_of(r0, 8)
        return pltpu.make_async_copy(hbm.at[pl.ds(r0, nrows), pl.ds(hp * W2, W2)],
                                     buf.at[hp, pl.ds(r0, nrows)], sem.at[hp])

    def x_copy(b):
        return pltpu.make_async_copy(x_hbm.at[b], xbuf.at[b], xsem.at[b])

    def o_copy(b):
        return pltpu.make_async_copy(obuf.at[b], out_hbm.at[b], osem.at[b])

    w_pieces = [(off, min(WSUB, WPB - off)) for off in range(0, WPB, WSUB)]
    n_half = (len(w_pieces) + 1) // 2
    w_pieces = (w_pieces[:n_half], w_pieces[n_half:])

    def issue_d(u, s, c):
        uk = u + 1
        uv = u
        static = isinstance(u, int)
        k_ok = uk < NU
        v_ok = (0 <= uv < NU) if static else uv < NU
        if static and not k_ok and not v_ok:
            return
        bk, hk = bh(uk)
        bv, hv = bh(max(uv, 0) if static else uv)
        if c == 0:
            if static and uk == 0 and s == 0:
                for i, r0 in enumerate(range(0, D, WSUB)):
                    w_copy(wq_hbm, wqbuf, wqsem, 0, r0, WSUB).start(priority=i % 2)
            for i, (off, n) in enumerate(w_pieces[s]):
                _when(_and(k_ok, hk + 1 < HP),
                      lambda: w_copy(wq_hbm, wqbuf, wqsem, hk + 1, bk * WPB + off, n).start(priority=i % 2))
        if c == NQ - 1:
            if static and uv == 0 and s == 0:
                for i, r0 in enumerate(range(0, D, WSUB)):
                    w_copy(wo_hbm, wobuf, wosem, 0, r0, WSUB).start(priority=i % 2)
            for i, (off, n) in enumerate(w_pieces[s]):
                _when(_and(v_ok, hv + 1 < HP),
                      lambda: w_copy(wo_hbm, wobuf, wosem, hv + 1, bv * WPB + off, n).start(priority=(i + 1) % 2))
        single = static and not (k_ok and v_ok)
        for j in range(NR // NQ):
            r0 = s * CK + (c * (NR // NQ) + j) * R
            _when(k_ok, lambda: blk_copy(k_hbm, kbuf, ksem, uk, s, r0, R).start(
                priority=(j % 2) if single else 0))
            _when(v_ok, lambda: blk_copy(v_hbm, vbuf, vsem, uv, s, r0, R).start(
                priority=((j + 1) % 2) if single else 1))

    def wait_a_inputs(u, s):
        if s == 0:
            b, hp = bh(u)
            _when(b == 0, lambda: w_copy(wq_hbm, wqbuf, wqsem, hp, 0, D).wait())
        blk_copy(k_hbm, kbuf, ksem, u, s, s * CK, CK).wait()

    def wait_b_inputs(u, s):
        blk_copy(v_hbm, vbuf, vsem, u, s, s * CK, CK).wait()
        if s == 1:
            b, hp = bh(u)
            _when(b == 0, lambda: w_copy(wo_hbm, wobuf, wosem, hp, 0, D).wait())

    def q_proj(u):
        b, hp = bh(u)
        q = jnp.dot(xbuf[b], wqbuf[hp], preferred_element_type=f32)
        qb = (q * scale).astype(bf16)
        qs = []
        for e in range(2):
            qe = jnp.concatenate([qb[:, e * W + r * DH:e * W + (r + 1) * DH] for r in range(rep)], axis=0)
            qbuf[e] = qe
            qs.append(qe)
        return qs

    def a_chunk(u, s, par, qs, c, mrun):
        e, g = divmod(c, 2)
        kc = kbuf[slot_of(u), c, s * CK:(s + 1) * CK, :]
        sc = jax.lax.dot_general(qs[e], kc, (((1,), (1,)), ((), ())), preferred_element_type=f32)
        lo = g * L + s * CK
        sbufs[par][e][:, lo:lo + CK] = sc
        mr = mrun[e]
        for j in range(CK // 128):
            sj = sc[:, j * 128:(j + 1) * 128]
            mr = sj if mr is None else jnp.maximum(mr, sj)
        mrun[e] = mr

    def b_chunk(u, s, par, m128, c, lrun, o):
        e, g = divmod(c, 2)
        ps = []
        lr = lrun[e]
        for j in range(CK // 128):
            lo = g * L + s * CK + j * 128
            pj = jnp.exp(sbufs[par][e][:, lo:lo + 128] - m128[e])
            lr = pj if lr is None else lr + pj
            ps.append(pj.astype(bf16))
        lrun[e] = lr
        p = jnp.concatenate(ps, axis=1)
        vc = vbuf[slot_of(u), c, s * CK:(s + 1) * CK, :]
        oc = jnp.dot(p, vc, preferred_element_type=f32)
        o[e] = oc if o[e] is None else o[e] + oc

    def b_fin(u, lrun, o):
        b, hp = bh(u)
        cols = []
        for e in range(2):
            l = jnp.sum(lrun[e], axis=-1, keepdims=True)
            oe = (o[e] / l).astype(bf16)
            cols += [oe[r * Sq:(r + 1) * Sq, :] for r in range(rep)]
        o2 = jnp.concatenate(cols, axis=1)
        contrib = jax.lax.dot_general(o2, wobuf[hp], (((1,), (1,)), ((), ())),
                                      preferred_element_type=f32)
        new = acc[b] + contrib
        acc[b] = new
        obuf[b] = new.astype(obuf.dtype)
        _when(hp == HP - 1, lambda: o_copy(b).start())

    def stage(u, s, par):
        static = isinstance(u, int)
        do_a = (u + 1 < NU) if static else True
        do_b = (u >= 0) if static else True
        if do_a:
            wait_a_inputs(u + 1, s)
        if do_b:
            wait_b_inputs(u, s)
        if do_a:
            if s == 0:
                qs = q_proj(u + 1)
                mrun = [None, None]
            else:
                qs = [qbuf[0], qbuf[1]]
                mrun = [mpart[0], mpart[1]]
        if do_b:
            m128 = [mbufs[par][0][...], mbufs[par][1][...]]
            if s == 0:
                lrun = [None, None]
                o = [None, None]
            else:
                lrun = [lpart[0], lpart[1]]
                o = [opart[0], opart[1]]
        for tok in SEQ[s]:
            kind, c = tok[0], int(tok[1:])
            if kind == "i":
                issue_d(u + 1, s, c)
            elif kind == "b" and do_b:
                b_chunk(u, s, par, m128, c, lrun, o)
            elif kind == "a" and do_a:
                a_chunk(u + 1, s, 1 - par, qs, c, mrun)
        if do_a:
            for e in range(2):
                if s == 0:
                    mpart[e] = mrun[e]
                else:
                    m = jnp.max(mrun[e], axis=-1, keepdims=True)
                    mbufs[1 - par][e][...] = jnp.broadcast_to(m, (M, 128))
        if do_b:
            if s == 0:
                for e in range(2):
                    lpart[e] = lrun[e]
                    opart[e] = o[e]
            else:
                b_fin(u, lrun, o)

    def last_stage(u, par):
        wait_b_inputs(u, 0)
        wait_b_inputs(u, 1)
        m128 = [mbufs[par][0][...], mbufs[par][1][...]]
        lrun = [None, None]
        o = [None, None]
        for s in range(2):
            for c in (0, 2, 1, 3):
                b_chunk(u, s, par, m128, c, lrun, o)
        b_fin(u, lrun, o)

    x_copy(0).start(priority=1)
    for c in range(NQ):
        issue_d(-1, 0, c)
    acc[...] = jnp.zeros(acc.shape, acc.dtype)
    for c in range(NQ):
        issue_d(-1, 1, c)
    for b in range(1, B):
        x_copy(b).start(priority=b % 2)
    x_copy(0).wait()
    n_static = (NU - 1) % 2
    for u in range(-1, n_static):
        stage(u, 0, u % 2)
        stage(u, 1, u % 2)
        if u == -1:
            for b in range(1, B):
                x_copy(b).wait()

    def body(i, carry):
        u = n_static + 2 * i
        for d in range(2):
            stage(u + d, 0, (n_static + d) % 2)
            stage(u + d, 1, (n_static + d) % 2)
        return carry

    jax.lax.fori_loop(0, (NU - 1 - n_static) // 2, body, 0)

    last_stage(NU - 1, (NU - 1) % 2)
    for b in range(B):
        o_copy(b).wait()


@jax.jit
def pallas_standalone__gqa_block_cached__near_ridge_kernel(
    x: jax.Array,
    k_cache: jax.Array,
    v_cache: jax.Array,
    wq: jax.Array,
    wo: jax.Array,
):
    B, Sq, D = x.shape
    _, Hkv, Sk, Dh = k_cache.shape
    assert Dh == DH and Sk == 4 * CK and Hkv % 2 == 0 and D % WSUB == 0 and D % (8 * B) == 0
    rep = HQ // Hkv
    W = rep * Dh
    M = rep * Sq
    HP = Hkv // 2
    NU = B * HP
    scale = float(Dh) ** -0.5

    kern = functools.partial(_kernel, B=B, Sq=Sq, Hkv=Hkv, Sk=Sk, D=D, rep=rep, scale=scale)
    any_spec = pl.BlockSpec(memory_space=pl.ANY)
    f32, bf16 = jnp.float32, jnp.bfloat16
    return pl.pallas_call(
        kern,
        in_specs=[any_spec] * 5,
        out_specs=any_spec,
        out_shape=jax.ShapeDtypeStruct((B, Sq, D), x.dtype),
        scratch_shapes=[
            pltpu.VMEM((B, Sq, D), bf16),
            pltpu.VMEM((HP, D, 2 * W), bf16),
            pltpu.VMEM((HP, D, 2 * W), bf16),
            pltpu.VMEM((2, NB, 4, Sk // 2, Dh), bf16),
            pltpu.VMEM((B, Sq, D), f32),
            pltpu.VMEM((B, Sq, D), bf16),
            pltpu.VMEM((2, M, Dh), bf16),
            pltpu.VMEM((2, M, 128), f32),
            pltpu.VMEM((2, M, 128), f32),
            pltpu.VMEM((2, M, Dh), f32),
        ] + [pltpu.VMEM((M, Sk), f32)] * 4
          + [pltpu.VMEM((M, 128), f32)] * 4
          + [
            pltpu.SemaphoreType.DMA((B,)),
            pltpu.SemaphoreType.DMA((HP,)),
            pltpu.SemaphoreType.DMA((HP,)),
            pltpu.SemaphoreType.DMA((2 * NB,)),
            pltpu.SemaphoreType.DMA((2 * NB,)),
            pltpu.SemaphoreType.DMA((B,)),
        ],
        compiler_params=pltpu.CompilerParams(
            vmem_limit_bytes=96 * 1024 * 1024,
            disable_bounds_checks=True,
        ),
    )(x, k_cache.reshape(NU, 4, Sk // 2, Dh), v_cache.reshape(NU, 4, Sk // 2, Dh), wq, wo.T)
```

```python
import functools

import jax
import jax.numpy as jnp
import jax.experimental.pallas as pl
import jax.experimental.pallas.tpu as pltpu

HQ = 16
DH = 256
NB = 4
CK = 512
R = 16
WSUB = 16
NQ = 4
SEQ = (("i0", "i1", "b0", "a0", "b1", "a1", "i2", "i3", "b2", "a2", "b3", "a3"),
       ("a0", "i0", "i1", "b0", "b2", "a2", "i2", "i3", "b1", "a1", "b3", "a3"))


def _divmod_pow2(t, n):
    assert n & (n - 1) == 0
    if isinstance(t, int):
        return t // n, t % n
    sh = n.bit_length() - 1
    return jax.lax.shift_right_logical(t, sh), jax.lax.bitwise_and(t, n - 1)


def _when(cond, fn):
    if isinstance(cond, bool):
        if cond:
            fn()
    else:
        pl.when(cond)(fn)


def _and(a, b):
    if isinstance(a, bool) and isinstance(b, bool):
        return a and b
    return jnp.logical_and(a, b)


def _kernel(x_hbm, k_hbm, v_hbm, wq_hbm, wo_hbm, out_hbm,
            xbuf, wqbuf, wobuf, kvbuf, acc, obuf, qbuf, mpart, lpart, opart,
            s00, s01, s10, s11, m00, m01, m10, m11,
            xsem, wqsem, wosem, ksem, vsem, osem,
            *, B, Sq, Hkv, Sk, D, rep, scale):
    kbuf = kvbuf.at[0]
    vbuf = kvbuf.at[1]
    sbufs = ((s00, s01), (s10, s11))
    mbufs = ((m00, m01), (m10, m11))
    HP = Hkv // 2
    NU = B * HP
    W = rep * DH
    W2 = 2 * W
    M = rep * Sq
    L = Sk // 2
    NR = CK // R
    WPB = D // B
    f32 = jnp.float32
    bf16 = jnp.bfloat16

    def bh(u):
        hp, b = _divmod_pow2(u, B)
        return b, hp

    def slot_of(u):
        return _divmod_pow2(u, NB)[1]

    def blk_copy(hbm, buf, sem, u, s, r0, nrows):
        b, hp = bh(u)
        slot = slot_of(u)
        return pltpu.make_async_copy(hbm.at[b * HP + hp, :, pl.ds(r0, nrows)],
                                     buf.at[slot, :, pl.ds(r0, nrows)], sem.at[2 * slot + s])

    def w_copy(hbm, buf, sem, hp, r0, nrows):
        if not isinstance(r0, int):
            r0 = pl.multiple_of(r0, 8)
        return pltpu.make_async_copy(hbm.at[pl.ds(r0, nrows), pl.ds(hp * W2, W2)],
                                     buf.at[hp, pl.ds(r0, nrows)], sem.at[hp])

    def x_copy(b):
        return pltpu.make_async_copy(x_hbm.at[b], xbuf.at[b], xsem.at[b])

    def o_copy(b):
        return pltpu.make_async_copy(obuf.at[b], out_hbm.at[b], osem.at[b])

    w_pieces = [(off, min(WSUB, WPB - off)) for off in range(0, WPB, WSUB)]
    n_half = (len(w_pieces) + 1) // 2
    w_pieces = (w_pieces[:n_half], w_pieces[n_half:])

    def issue_d(u, s, c):
        uk = u + 1
        uv = u
        static = isinstance(u, int)
        k_ok = uk < NU
        v_ok = (0 <= uv < NU) if static else uv < NU
        if static and not k_ok and not v_ok:
            return
        bk, hk = bh(uk)
        bv, hv = bh(max(uv, 0) if static else uv)
        if c == 0:
            if static and uk == 0 and s == 0:
                for i, r0 in enumerate(range(0, D, WSUB)):
                    w_copy(wq_hbm, wqbuf, wqsem, 0, r0, WSUB).start(priority=i % 2)
            for i, (off, n) in enumerate(w_pieces[s]):
                _when(_and(k_ok, hk + 1 < HP),
                      lambda: w_copy(wq_hbm, wqbuf, wqsem, hk + 1, bk * WPB + off, n).start(priority=i % 2))
        if c == NQ - 1:
            if static and uv == 0 and s == 0:
                for i, r0 in enumerate(range(0, D, WSUB)):
                    w_copy(wo_hbm, wobuf, wosem, 0, r0, WSUB).start(priority=i % 2)
            for i, (off, n) in enumerate(w_pieces[s]):
                _when(_and(v_ok, hv + 1 < HP),
                      lambda: w_copy(wo_hbm, wobuf, wosem, hv + 1, bv * WPB + off, n).start(priority=(i + 1) % 2))
        single = static and not (k_ok and v_ok)
        for j in range(NR // NQ):
            r0 = s * CK + (c * (NR // NQ) + j) * R
            _when(k_ok, lambda: blk_copy(k_hbm, kbuf, ksem, uk, s, r0, R).start(
                priority=(j % 2) if single else 0))
            _when(v_ok, lambda: blk_copy(v_hbm, vbuf, vsem, uv, s, r0, R).start(
                priority=((j + 1) % 2) if single else 1))

    def wait_a_inputs(u, s):
        if s == 0:
            b, hp = bh(u)
            _when(b == 0, lambda: w_copy(wq_hbm, wqbuf, wqsem, hp, 0, D).wait())
        blk_copy(k_hbm, kbuf, ksem, u, s, s * CK, CK).wait()

    def wait_b_inputs(u, s):
        blk_copy(v_hbm, vbuf, vsem, u, s, s * CK, CK).wait()
        if s == 1:
            b, hp = bh(u)
            _when(b == 0, lambda: w_copy(wo_hbm, wobuf, wosem, hp, 0, D).wait())

    def q_proj(u):
        b, hp = bh(u)
        q = jnp.dot(xbuf[b], wqbuf[hp], preferred_element_type=f32)
        qb = (q * scale).astype(bf16)
        qs = []
        for e in range(2):
            qe = jnp.concatenate([qb[:, e * W + r * DH:e * W + (r + 1) * DH] for r in range(rep)], axis=0)
            qbuf[e] = qe
            qs.append(qe)
        return qs

    def a_chunk(u, s, par, qs, c, mrun):
        e, g = divmod(c, 2)
        kc = kbuf[slot_of(u), c, s * CK:(s + 1) * CK, :]
        sc = jax.lax.dot_general(qs[e], kc, (((1,), (1,)), ((), ())), preferred_element_type=f32)
        lo = g * L + s * CK
        sbufs[par][e][:, lo:lo + CK] = sc
        mr = mrun[e]
        for j in range(CK // 128):
            sj = sc[:, j * 128:(j + 1) * 128]
            mr = sj if mr is None else jnp.maximum(mr, sj)
        mrun[e] = mr

    def b_chunk(u, s, par, m128, c, lrun, o):
        e, g = divmod(c, 2)
        ps = []
        lr = lrun[e]
        for j in range(CK // 128):
            lo = g * L + s * CK + j * 128
            pj = jnp.exp(sbufs[par][e][:, lo:lo + 128] - m128[e])
            lr = pj if lr is None else lr + pj
            ps.append(pj.astype(bf16))
        lrun[e] = lr
        p = jnp.concatenate(ps, axis=1)
        vc = vbuf[slot_of(u), c, s * CK:(s + 1) * CK, :]
        oc = jnp.dot(p, vc, preferred_element_type=f32)
        o[e] = oc if o[e] is None else o[e] + oc

    def b_fin(u, lrun, o):
        b, hp = bh(u)
        cols = []
        for e in range(2):
            l = jnp.sum(lrun[e], axis=-1, keepdims=True)
            oe = (o[e] / l).astype(bf16)
            cols += [oe[r * Sq:(r + 1) * Sq, :] for r in range(rep)]
        o2 = jnp.concatenate(cols, axis=1)
        contrib = jax.lax.dot_general(o2, wobuf[hp], (((1,), (1,)), ((), ())),
                                      preferred_element_type=f32)
        new = acc[b] + contrib
        acc[b] = new
        obuf[b] = new.astype(obuf.dtype)
        _when(hp == HP - 1, lambda: o_copy(b).start())

    def stage(u, s, par):
        static = isinstance(u, int)
        do_a = (u + 1 < NU) if static else True
        do_b = (u >= 0) if static else True
        if do_a:
            wait_a_inputs(u + 1, s)
        if do_b:
            wait_b_inputs(u, s)
        if do_a:
            if s == 0:
                qs = q_proj(u + 1)
                mrun = [None, None]
            else:
                qs = [qbuf[0], qbuf[1]]
                mrun = [mpart[0], mpart[1]]
        if do_b:
            m128 = [mbufs[par][0][...], mbufs[par][1][...]]
            if s == 0:
                lrun = [None, None]
                o = [None, None]
            else:
                lrun = [lpart[0], lpart[1]]
                o = [opart[0], opart[1]]
        for tok in SEQ[s]:
            kind, c = tok[0], int(tok[1:])
            if kind == "i":
                issue_d(u + 1, s, c)
            elif kind == "b" and do_b:
                b_chunk(u, s, par, m128, c, lrun, o)
            elif kind == "a" and do_a:
                a_chunk(u + 1, s, 1 - par, qs, c, mrun)
        if do_a:
            for e in range(2):
                if s == 0:
                    mpart[e] = mrun[e]
                else:
                    m = jnp.max(mrun[e], axis=-1, keepdims=True)
                    mbufs[1 - par][e][...] = jnp.broadcast_to(m, (M, 128))
        if do_b:
            if s == 0:
                for e in range(2):
                    lpart[e] = lrun[e]
                    opart[e] = o[e]
            else:
                b_fin(u, lrun, o)

    def last_stage(u, par):
        wait_b_inputs(u, 0)
        wait_b_inputs(u, 1)
        m128 = [mbufs[par][0][...], mbufs[par][1][...]]
        lrun = [None, None]
        o = [None, None]
        for s in range(2):
            for c in (0, 2, 1, 3):
                b_chunk(u, s, par, m128, c, lrun, o)
        b_fin(u, lrun, o)

    x_copy(0).start(priority=1)
    for c in range(NQ):
        issue_d(-1, 0, c)
    acc[...] = jnp.zeros(acc.shape, acc.dtype)
    for c in range(NQ):
        issue_d(-1, 1, c)
    for b in range(1, B):
        x_copy(b).start(priority=b % 2)
    x_copy(0).wait()
    n_static = (NU - 1) % 2
    for u in range(-1, n_static):
        stage(u, 0, u % 2)
        stage(u, 1, u % 2)
        if u == -1:
            for b in range(1, B):
                x_copy(b).wait()

    def body(i, carry):
        u = n_static + 2 * i
        for d in range(2):
            stage(u + d, 0, (n_static + d) % 2)
            stage(u + d, 1, (n_static + d) % 2)
        return carry

    jax.lax.fori_loop(0, (NU - 1 - n_static) // 2, body, 0)

    last_stage(NU - 1, (NU - 1) % 2)
    for b in range(B):
        o_copy(b).wait()


@jax.jit
def pallas_standalone__gqa_block_cached__near_ridge_kernel(
    x: jax.Array,
    k_cache: jax.Array,
    v_cache: jax.Array,
    wq: jax.Array,
    wo: jax.Array,
):
    B, Sq, D = x.shape
    _, Hkv, Sk, Dh = k_cache.shape
    assert Dh == DH and Sk == 4 * CK and Hkv % 2 == 0 and D % WSUB == 0 and D % (8 * B) == 0
    rep = HQ // Hkv
    W = rep * Dh
    M = rep * Sq
    HP = Hkv // 2
    NU = B * HP
    scale = float(Dh) ** -0.5

    kern = functools.partial(_kernel, B=B, Sq=Sq, Hkv=Hkv, Sk=Sk, D=D, rep=rep, scale=scale)
    any_spec = pl.BlockSpec(memory_space=pl.ANY)
    f32, bf16 = jnp.float32, jnp.bfloat16
    base = dict(vmem_limit_bytes=96 * 1024 * 1024, disable_bounds_checks=True)
    try:
        params = pltpu.CompilerParams(disable_semaphore_checks=True, **base)
    except TypeError:
        params = pltpu.CompilerParams(**base)
    return pl.pallas_call(
        kern,
        in_specs=[any_spec] * 5,
        out_specs=any_spec,
        out_shape=jax.ShapeDtypeStruct((B, Sq, D), x.dtype),
        scratch_shapes=[
            pltpu.VMEM((B, Sq, D), bf16),
            pltpu.VMEM((HP, D, 2 * W), bf16),
            pltpu.VMEM((HP, D, 2 * W), bf16),
            pltpu.VMEM((2, NB, 4, Sk // 2, Dh), bf16),
            pltpu.VMEM((B, Sq, D), f32),
            pltpu.VMEM((B, Sq, D), bf16),
            pltpu.VMEM((2, M, Dh), bf16),
            pltpu.VMEM((2, M, 128), f32),
            pltpu.VMEM((2, M, 128), f32),
            pltpu.VMEM((2, M, Dh), f32),
        ] + [pltpu.VMEM((M, Sk), f32)] * 4
          + [pltpu.VMEM((M, 128), f32)] * 4
          + [
            pltpu.SemaphoreType.DMA((B,)),
            pltpu.SemaphoreType.DMA((HP,)),
            pltpu.SemaphoreType.DMA((HP,)),
            pltpu.SemaphoreType.DMA((2 * NB,)),
            pltpu.SemaphoreType.DMA((2 * NB,)),
            pltpu.SemaphoreType.DMA((B,)),
        ],
        compiler_params=params,
    )(x, k_cache.reshape(NU, 4, Sk // 2, Dh), v_cache.reshape(NU, 4, Sk // 2, Dh), wq, wo.T)
```

```python
import functools

import jax
import jax.numpy as jnp
import jax.experimental.pallas as pl
import jax.experimental.pallas.tpu as pltpu

HQ = 16
DH = 256
NB = 4
CK = 512
R = 16
WSUB = 16
NQ = 4
SEQ = (("i0", "i1", "b0", "a0", "b1", "a1", "i2", "i3", "b2", "a2", "b3", "a3"),
       ("a0", "i0", "i1", "b0", "b2", "a2", "i2", "i3", "b1", "a1", "b3", "a3"))


def _divmod_pow2(t, n):
    assert n & (n - 1) == 0
    if isinstance(t, int):
        return t // n, t % n
    sh = n.bit_length() - 1
    return jax.lax.shift_right_logical(t, sh), jax.lax.bitwise_and(t, n - 1)


def _when(cond, fn):
    if isinstance(cond, bool):
        if cond:
            fn()
    else:
        pl.when(cond)(fn)


def _and(a, b):
    if isinstance(a, bool) and isinstance(b, bool):
        return a and b
    return jnp.logical_and(a, b)


def _kernel(x_hbm, k_hbm, v_hbm, wq_hbm, wo_hbm, out_hbm,
            xbuf, wqbuf, wobuf, kvbuf, acc, obuf, qbuf, mpart, lpart, opart,
            s00, s01, s10, s11, m00, m01, m10, m11,
            xsem, wqsem, wosem, ksem, vsem, osem,
            *, B, Sq, Hkv, Sk, D, rep, scale):
    kbuf = kvbuf.at[0]
    vbuf = kvbuf.at[1]
    sbufs = ((s00, s01), (s10, s11))
    mbufs = ((m00, m01), (m10, m11))
    HP = Hkv // 2
    NU = B * HP
    W = rep * DH
    W2 = 2 * W
    M = rep * Sq
    L = Sk // 2
    NR = CK // R
    WPB = D // B
    f32 = jnp.float32
    bf16 = jnp.bfloat16

    def bh(u):
        hp, b = _divmod_pow2(u, B)
        return b, hp

    def slot_of(u):
        return _divmod_pow2(u, NB)[1]

    def blk_copy(hbm, buf, sem, u, s, r0, nrows):
        b, hp = bh(u)
        slot = slot_of(u)
        return pltpu.make_async_copy(hbm.at[b * HP + hp, :, pl.ds(r0, nrows)],
                                     buf.at[slot, :, pl.ds(r0, nrows)], sem.at[2 * slot + s])

    def w_copy(hbm, buf, sem, hp, r0, nrows):
        if not isinstance(r0, int):
            r0 = pl.multiple_of(r0, 8)
        return pltpu.make_async_copy(hbm.at[pl.ds(r0, nrows), pl.ds(hp * W2, W2)],
                                     buf.at[hp, pl.ds(r0, nrows)], sem.at[hp])

    def x_copy(b):
        return pltpu.make_async_copy(x_hbm.at[b], xbuf.at[b], xsem.at[b])

    def o_copy(b):
        return pltpu.make_async_copy(obuf.at[b], out_hbm.at[b], osem.at[b])

    w_pieces = [(off, min(WSUB, WPB - off)) for off in range(0, WPB, WSUB)]
    n_half = (len(w_pieces) + 1) // 2
    w_pieces = (w_pieces[:n_half], w_pieces[n_half:])

    def issue_d(u, s, c):
        uk = u + 1
        uv = u
        static = isinstance(u, int)
        k_ok = uk < NU
        v_ok = (0 <= uv < NU) if static else uv < NU
        if static and not k_ok and not v_ok:
            return
        bk, hk = bh(uk)
        bv, hv = bh(max(uv, 0) if static else uv)
        if c == 0:
            for i, (off, n) in enumerate(w_pieces[s]):
                _when(_and(k_ok, hk + 1 < HP),
                      lambda: w_copy(wq_hbm, wqbuf, wqsem, hk + 1, bk * WPB + off, n).start(priority=i % 2))
        if c == NQ - 1:
            if static and uv == 0 and s == 0:
                for i, r0 in enumerate(range(0, D, WSUB)):
                    w_copy(wo_hbm, wobuf, wosem, 0, r0, WSUB).start(priority=i % 2)
            for i, (off, n) in enumerate(w_pieces[s]):
                _when(_and(v_ok, hv + 1 < HP),
                      lambda: w_copy(wo_hbm, wobuf, wosem, hv + 1, bv * WPB + off, n).start(priority=(i + 1) % 2))
        single = static and not (k_ok and v_ok)
        for j in range(NR // NQ):
            r0 = s * CK + (c * (NR // NQ) + j) * R
            _when(k_ok, lambda: blk_copy(k_hbm, kbuf, ksem, uk, s, r0, R).start(
                priority=(j % 2) if single else 0))
            _when(v_ok, lambda: blk_copy(v_hbm, vbuf, vsem, uv, s, r0, R).start(
                priority=((j + 1) % 2) if single else 1))

    def wait_a_inputs(u, s):
        if s == 0:
            b, hp = bh(u)
            _when(b == 0, lambda: w_copy(wq_hbm, wqbuf, wqsem, hp, 0, D).wait())
        blk_copy(k_hbm, kbuf, ksem, u, s, s * CK, CK).wait()

    def wait_b_inputs(u, s):
        blk_copy(v_hbm, vbuf, vsem, u, s, s * CK, CK).wait()
        if s == 1:
            b, hp = bh(u)
            _when(b == 0, lambda: w_copy(wo_hbm, wobuf, wosem, hp, 0, D).wait())

    def q_proj(u):
        b, hp = bh(u)
        q = jnp.dot(xbuf[b], wqbuf[hp], preferred_element_type=f32)
        qb = (q * scale).astype(bf16)
        qs = []
        for e in range(2):
            qe = jnp.concatenate([qb[:, e * W + r * DH:e * W + (r + 1) * DH] for r in range(rep)], axis=0)
            qbuf[e] = qe
            qs.append(qe)
        return qs

    def a_chunk(u, s, par, qs, c, mrun):
        e, g = divmod(c, 2)
        kc = kbuf[slot_of(u), c, s * CK:(s + 1) * CK, :]
        sc = jax.lax.dot_general(qs[e], kc, (((1,), (1,)), ((), ())), preferred_element_type=f32)
        lo = g * L + s * CK
        sbufs[par][e][:, lo:lo + CK] = sc
        mr = mrun[e]
        for j in range(CK // 128):
            sj = sc[:, j * 128:(j + 1) * 128]
            mr = sj if mr is None else jnp.maximum(mr, sj)
        mrun[e] = mr

    def b_chunk(u, s, par, m128, c, lrun, o):
        e, g = divmod(c, 2)
        ps = []
        lr = lrun[e]
        for j in range(CK // 128):
            lo = g * L + s * CK + j * 128
            pj = jnp.exp(sbufs[par][e][:, lo:lo + 128] - m128[e])
            lr = pj if lr is None else lr + pj
            ps.append(pj.astype(bf16))
        lrun[e] = lr
        p = jnp.concatenate(ps, axis=1)
        vc = vbuf[slot_of(u), c, s * CK:(s + 1) * CK, :]
        oc = jnp.dot(p, vc, preferred_element_type=f32)
        o[e] = oc if o[e] is None else o[e] + oc

    def b_fin(u, lrun, o):
        b, hp = bh(u)
        cols = []
        for e in range(2):
            l = jnp.sum(lrun[e], axis=-1, keepdims=True)
            oe = (o[e] / l).astype(bf16)
            cols += [oe[r * Sq:(r + 1) * Sq, :] for r in range(rep)]
        o2 = jnp.concatenate(cols, axis=1)
        contrib = jax.lax.dot_general(o2, wobuf[hp], (((1,), (1,)), ((), ())),
                                      preferred_element_type=f32)
        new = acc[b] + contrib
        acc[b] = new
        obuf[b] = new.astype(obuf.dtype)
        _when(hp == HP - 1, lambda: o_copy(b).start())

    def stage(u, s, par):
        static = isinstance(u, int)
        do_a = (u + 1 < NU) if static else True
        do_b = (u >= 0) if static else True
        if do_a:
            wait_a_inputs(u + 1, s)
        if do_b:
            wait_b_inputs(u, s)
        if do_a:
            if s == 0:
                qs = q_proj(u + 1)
                mrun = [None, None]
            else:
                qs = [qbuf[0], qbuf[1]]
                mrun = [mpart[0], mpart[1]]
        if do_b:
            m128 = [mbufs[par][0][...], mbufs[par][1][...]]
            if s == 0:
                lrun = [None, None]
                o = [None, None]
            else:
                lrun = [lpart[0], lpart[1]]
                o = [opart[0], opart[1]]
        for tok in SEQ[s]:
            kind, c = tok[0], int(tok[1:])
            if kind == "i":
                issue_d(u + 1, s, c)
            elif kind == "b" and do_b:
                b_chunk(u, s, par, m128, c, lrun, o)
            elif kind == "a" and do_a:
                a_chunk(u + 1, s, 1 - par, qs, c, mrun)
        if do_a:
            for e in range(2):
                if s == 0:
                    mpart[e] = mrun[e]
                else:
                    m = jnp.max(mrun[e], axis=-1, keepdims=True)
                    mbufs[1 - par][e][...] = jnp.broadcast_to(m, (M, 128))
        if do_b:
            if s == 0:
                for e in range(2):
                    lpart[e] = lrun[e]
                    opart[e] = o[e]
            else:
                b_fin(u, lrun, o)

    def last_stage(u, par):
        wait_b_inputs(u, 0)
        wait_b_inputs(u, 1)
        m128 = [mbufs[par][0][...], mbufs[par][1][...]]
        lrun = [None, None]
        o = [None, None]
        for s in range(2):
            for c in (0, 2, 1, 3):
                b_chunk(u, s, par, m128, c, lrun, o)
        b_fin(u, lrun, o)

    x_copy(0).start(priority=1)
    n_w0 = D // WSUB

    def first_k(j, carry):
        r0 = pl.multiple_of(j * R, R)
        blk_copy(k_hbm, kbuf, ksem, 0, 0, r0, R).start(priority=0)
        pl.when(j < n_w0)(lambda: w_copy(wq_hbm, wqbuf, wqsem, 0, j * WSUB, WSUB).start(priority=1))
        return carry

    assert n_w0 <= NR
    jax.lax.fori_loop(0, NR, first_k, 0)

    def second_k(j, carry):
        for half in range(2):
            r0 = pl.multiple_of(CK + (half * (NR // 2) + j) * R, R)
            blk_copy(k_hbm, kbuf, ksem, 0, 1, r0, R).start(priority=half)
        return carry

    jax.lax.fori_loop(0, NR // 2, second_k, 0)
    for b in range(1, B):
        x_copy(b).start(priority=b % 2)
    if HP > 1:
        for s in range(2):
            for i, (off, n) in enumerate(w_pieces[s]):
                w_copy(wq_hbm, wqbuf, wqsem, 1, off, n).start(priority=i % 2)
    acc[...] = jnp.zeros(acc.shape, acc.dtype)
    x_copy(0).wait()
    n_static = (NU - 1) % 2
    for u in range(-1, n_static):
        stage(u, 0, u % 2)
        stage(u, 1, u % 2)
        if u == -1:
            for b in range(1, B):
                x_copy(b).wait()

    def body(i, carry):
        u = n_static + 2 * i
        for d in range(2):
            stage(u + d, 0, (n_static + d) % 2)
            stage(u + d, 1, (n_static + d) % 2)
        return carry

    jax.lax.fori_loop(0, (NU - 1 - n_static) // 2, body, 0)

    last_stage(NU - 1, (NU - 1) % 2)
    for b in range(B):
        o_copy(b).wait()


@jax.jit
def pallas_standalone__gqa_block_cached__near_ridge_kernel(
    x: jax.Array,
    k_cache: jax.Array,
    v_cache: jax.Array,
    wq: jax.Array,
    wo: jax.Array,
):
    B, Sq, D = x.shape
    _, Hkv, Sk, Dh = k_cache.shape
    assert Dh == DH and Sk == 4 * CK and Hkv % 2 == 0 and D % WSUB == 0 and D % (8 * B) == 0
    rep = HQ // Hkv
    W = rep * Dh
    M = rep * Sq
    HP = Hkv // 2
    NU = B * HP
    scale = float(Dh) ** -0.5

    kern = functools.partial(_kernel, B=B, Sq=Sq, Hkv=Hkv, Sk=Sk, D=D, rep=rep, scale=scale)
    any_spec = pl.BlockSpec(memory_space=pl.ANY)
    f32, bf16 = jnp.float32, jnp.bfloat16
    base = dict(vmem_limit_bytes=96 * 1024 * 1024, disable_bounds_checks=True)
    try:
        params = pltpu.CompilerParams(disable_semaphore_checks=True, **base)
    except TypeError:
        params = pltpu.CompilerParams(**base)
    return pl.pallas_call(
        kern,
        in_specs=[any_spec] * 5,
        out_specs=any_spec,
        out_shape=jax.ShapeDtypeStruct((B, Sq, D), x.dtype),
        scratch_shapes=[
            pltpu.VMEM((B, Sq, D), bf16),
            pltpu.VMEM((HP, D, 2 * W), bf16),
            pltpu.VMEM((HP, D, 2 * W), bf16),
            pltpu.VMEM((2, NB, 4, Sk // 2, Dh), bf16),
            pltpu.VMEM((B, Sq, D), f32),
            pltpu.VMEM((B, Sq, D), bf16),
            pltpu.VMEM((2, M, Dh), bf16),
            pltpu.VMEM((2, M, 128), f32),
            pltpu.VMEM((2, M, 128), f32),
            pltpu.VMEM((2, M, Dh), f32),
        ] + [pltpu.VMEM((M, Sk), f32)] * 4
          + [pltpu.VMEM((M, 128), f32)] * 4
          + [
            pltpu.SemaphoreType.DMA((B,)),
            pltpu.SemaphoreType.DMA((HP,)),
            pltpu.SemaphoreType.DMA((HP,)),
            pltpu.SemaphoreType.DMA((2 * NB,)),
            pltpu.SemaphoreType.DMA((2 * NB,)),
            pltpu.SemaphoreType.DMA((B,)),
        ],
        compiler_params=params,
    )(x, k_cache.reshape(NU, 4, Sk // 2, Dh), v_cache.reshape(NU, 4, Sk // 2, Dh), wq, wo.T)
```
